```python
import os as _os
_os.environ.setdefault("JAX_PLATFORMS", "cpu")
import jax
import jax.numpy as jnp

def _softmax(x, axis=-1):
    return jax.nn.softmax(x, axis=axis)
def _gelu(x):
    return jax.nn.gelu(x, approximate=True)
def _silu(x):
    return jax.nn.silu(x)
def _sigmoid(x):
    return jax.nn.sigmoid(x)
def _layernorm(x, axis=-1, eps=1e-5):
    m = jnp.mean(x, axis=axis, keepdims=True)
    v = jnp.var(x, axis=axis, keepdims=True)
    return (x - m) / jnp.sqrt(v + eps)
def _scatter_add(tgt, idx, src, axis=0):
    return tgt.at[idx].add(src)
def _segment_sum(src, seg, n):
    return jax.ops.segment_sum(src, seg, n)
class _Rng:
    def __init__(self, key):
        self._k = key
    def _next(self):
        self._k, sub = jax.random.split(self._k)
        return sub
    def normal(self, shape):
        return jax.random.normal(self._next(), shape, dtype=jnp.bfloat16)
    def randint(self, lo, hi, shape):
        return jax.random.randint(self._next(), shape, lo, hi, dtype=jnp.int32)
    def uniform(self, shape, lo=0.0, hi=1.0):
        return jax.random.uniform(self._next(), shape, jnp.bfloat16, lo, hi)
    def permutation(self, n):
        return jax.random.permutation(self._next(), n)


kernel_name = 'concat_heads__spectral_gfnet__sliding_block__prompt'

def setup_inputs():
    _rng = _Rng(jax.random.key(int.from_bytes(__import__("os").urandom(4), "little")))
    _w = (lambda a: (lambda t: t.astype(jnp.bfloat16) if jnp.issubdtype(t.dtype, jnp.floating) else t)(jnp.asarray(a)))
    def _A_setup():
        B, S, D = 1, 2048, 640
        Df = D // 2 + 1
        return {
            "x": _w((lambda *s: _rng.normal(s) * 0.05)(B, S, D)),
            "w_r": _w((lambda *s: _rng.normal(s) * 0.4)(S, Df) * 0.02),
            "w_i": _w((lambda *s: _rng.normal(s) * 0.4)(S, Df) * 0.02),
        }
    _A_in = _A_setup()

    def _B_setup():
        B, S, D = 1, 2048, 640
        return {
            "x": _w((lambda *s: _rng.normal(s) * 0.2)(B, S, D)),
            "wqkv": _w((lambda *s: _rng.normal(s) * 0.2)(D, 3 * D)),
            "wo": _w((lambda *s: _rng.normal(s) * 0.05)(D, D)),
        }
    _B_in = _B_setup()

    return {
        "A_x": _A_in["x"],
        "A_w_r": _A_in["w_r"],
        "A_w_i": _A_in["w_i"],
        "B_x": _B_in["x"],
        "B_wqkv": _B_in["wqkv"],
        "B_wo": _B_in["wo"],
    }

def reference(A_x, A_w_r, A_w_i, B_x, B_wqkv, B_wo):
    def _A_ref(x, w_r, w_i):
        B, S, D = x.shape
        X = (lambda x, axes=(-2,-1): jnp.fft.rfft2(x.astype(jnp.float32), axes=axes))(x, axes=(-2, -1))
        W = w_r + 1j * w_i
        X = X * W
        y = (lambda x, s, axes=(-2,-1): jnp.fft.irfft2(x, s=s, axes=axes).astype(jnp.bfloat16))(X, (S, D), axes=(-2, -1))
        return y

    def _B_ref(x, wqkv, wo):
        B, S, D = x.shape
        H = 32; Dh = D // H; W = 256
        qkv = (lambda x, *d: x.transpose(*d))((x @ wqkv).reshape(B, S, 3, H, Dh), 2, 0, 3, 1, 4)
        q, k, v = qkv[0], qkv[1], qkv[2]
        scores = jnp.einsum("bhqd,bhkd->bhqk", q, k) * (Dh ** -0.5)
        idx = jnp.arange(S)
        mask = (idx[:, None] - idx[None, :] >= 0) & (idx[:, None] - idx[None, :] < W)
        scores = jnp.where(mask[None, None], scores, -1e9)
        p = _softmax(scores, axis=-1)
        o = jnp.einsum("bhqk,bhkd->bhqd", p, v)
        return (lambda x, *d: x.transpose(*d))(o, 0, 2, 1, 3).reshape(B, S, D) @ wo

    a = _A_ref(A_x, A_w_r, A_w_i)
    b = _B_ref(B_x, B_wqkv, B_wo)
    return jnp.concatenate([a, b], axis=-1)
```

```python
import math

import numpy as np
import jax
import jax.numpy as jnp
from jax.experimental import pallas as pl
from jax.experimental.pallas import tpu as pltpu

S = 2048
D = 640
DF = D // 2 + 1
DFP = 384
H = 32
DH = D // H
WIN = 256
QB = 128
NQB = S // QB
NT = D // 128
KW = WIN + QB
N1 = 16
N2 = 128
CH = 512
NCH = S // CH
NEG = -1e9
HP = 32

_UNITS = [[h for h in range(H) if DH * h < 128 * (t + 1) and DH * (h + 1) > 128 * t]
          for t in range(NT)]


def _make_consts():
    d = np.arange(D)[:, None]
    m = np.arange(DFP)[None, :]
    valid = m < DF
    ang = 2.0 * np.pi * ((d * m) % D) / D
    fd = np.concatenate([np.where(valid, np.cos(ang), 0.0),
                         np.where(valid, -np.sin(ang), 0.0)], axis=1)
    c = np.where((m == 0) | (m == D // 2), 1.0, 2.0) * valid
    sc = 1.0 / (D * S)
    gd = np.concatenate([(c * np.cos(ang) * sc).T,
                         (-c * np.sin(ang) * sc).T], axis=0)
    kb = np.arange(N2)[:, None]
    b = np.arange(N2)[None, :]
    a2 = 2.0 * np.pi * ((kb * b) % N2) / N2
    cr, sr = np.cos(a2), np.sin(a2)
    ff = np.block([[cr, sr], [-sr, cr]])
    fi = np.block([[cr, -sr], [sr, cr]])
    ka = np.arange(N1)[:, None]
    bb = np.arange(N2)[None, :]
    a3 = (2.0 * np.pi * (ka * bb) / S).reshape(S, 1)
    twr = np.broadcast_to(np.cos(a3), (S, 128))
    twi = np.broadcast_to(-np.sin(a3), (S, 128))
    return (jnp.asarray(fd, jnp.bfloat16), jnp.asarray(gd, jnp.bfloat16),
            jnp.asarray(ff, jnp.bfloat16), jnp.asarray(fi, jnp.bfloat16),
            jnp.asarray(twr, jnp.float32), jnp.asarray(twi, jnp.float32))


def _dft4(x, sign):
    (a0r, a0i), (a1r, a1i), (a2r, a2i), (a3r, a3i) = x
    s0r, s0i = a0r + a2r, a0i + a2i
    d0r, d0i = a0r - a2r, a0i - a2i
    s1r, s1i = a1r + a3r, a1i + a3i
    d1r, d1i = a1r - a3r, a1i - a3i
    if sign < 0:
        x1 = (d0r + d1i, d0i - d1r)
        x3 = (d0r - d1i, d0i + d1r)
    else:
        x1 = (d0r - d1i, d0i + d1r)
        x3 = (d0r + d1i, d0i - d1r)
    return [(s0r + s1r, s0i + s1i), x1, (s0r - s1r, s0i - s1i), x3]


def _cmul_const(xr, xi, e, sign):
    e = e % 16
    if e == 0:
        return xr, xi
    if e == 4:
        return (xi, -xr) if sign < 0 else (-xi, xr)
    ang = sign * 2.0 * math.pi * e / 16.0
    cr, ci = math.cos(ang), math.sin(ang)
    if e in (2, 6):
        r = abs(cr)
        sr = 1.0 if cr > 0 else -1.0
        si = 1.0 if ci > 0 else -1.0
        a = xr * r
        b_ = xi * r
        re = (a if sr > 0 else -a) - (b_ if si > 0 else -b_)
        im = (a if si > 0 else -a) + (b_ if sr > 0 else -b_)
        return re, im
    return xr * cr - xi * ci, xr * ci + xi * cr


def _dft16(x, sign):
    t = [_dft4([x[a0 + 4 * a1] for a1 in range(4)], sign) for a0 in range(4)]
    for a0 in range(1, 4):
        for k1 in range(1, 4):
            t[a0][k1] = _cmul_const(t[a0][k1][0], t[a0][k1][1], a0 * k1, sign)
    out = [None] * 16
    for k1 in range(4):
        u = _dft4([t[a0][k1] for a0 in range(4)], sign)
        for k0 in range(4):
            out[k1 + 4 * k0] = u[k0]
    return out


def _kernel(xb_hbm, wqkv_hbm, wo_hbm, xa_hbm, wr_hbm, wi_hbm,
            fd_hbm, gd_hbm, ff_hbm, fi_hbm, twr_hbm, twi_hbm,
            out_hbm,
            xb_v, wqkv_v, wo_v, xa_v, wr_v, wi_v, fd_v, gd_v, ff_v, fi_v, twr_v, twi_v,
            q_s, k_s, vt_s, ot_s, o_s, xd_s, v16_s, wt_s, wfr_s, wfi_s, sta_s, stb_s,
            isem, osem):
    f32 = jnp.float32
    bf16 = jnp.bfloat16

    copies = []

    def cp(src, dst):
        c = pltpu.make_async_copy(src, dst, isem.at[len(copies)])
        copies.append(c)
        return c

    c_wq = cp(wqkv_hbm.at[:, 0:D], wqkv_v.at[:, 0:D])
    c_xb = [cp(xb_hbm.at[pl.ds(0, CH), :], xb_v.at[pl.ds(0, CH), :])]
    c_wk = cp(wqkv_hbm.at[:, D:2 * D], wqkv_v.at[:, D:2 * D])
    c_wv = cp(wqkv_hbm.at[:, 2 * D:3 * D], wqkv_v.at[:, 2 * D:3 * D])
    for c in range(1, NCH):
        c_xb.append(cp(xb_hbm.at[pl.ds(c * CH, CH), :], xb_v.at[pl.ds(c * CH, CH), :]))
    c_wo = cp(wo_hbm, wo_v)
    c_fd = cp(fd_hbm, fd_v)
    c_xa = cp(xa_hbm, xa_v)
    c_twr = cp(twr_hbm, twr_v)
    c_twi = cp(twi_hbm, twi_v)
    c_ff = cp(ff_hbm, ff_v)
    c_fi = cp(fi_hbm, fi_v)
    c_wr = cp(wr_hbm, wr_v)
    c_wi = cp(wi_hbm, wi_v)
    c_gd = cp(gd_hbm, gd_v)
    for c in copies:
        c.start()

    out_copies = []

    k_s[0:WIN, :] = jnp.zeros((WIN, D), bf16)
    for j in range(WIN // 128):
        vt_s[j] = jnp.zeros((H * HP, 128), bf16)
    qscale = (DH ** -0.5) * math.log2(math.e)
    c_wq.wait()
    for c in range(NCH):
        c_xb[c].wait()
        x = xb_v[c * CH:(c + 1) * CH, :]
        q_s[c * CH:(c + 1) * CH, :] = qscale * jnp.dot(
            x, wqkv_v[:, 0:D], preferred_element_type=f32)
        if c == 0:
            c_wk.wait()
        k_s[WIN + c * CH:WIN + (c + 1) * CH, :] = jnp.dot(
            x, wqkv_v[:, D:2 * D], preferred_element_type=f32).astype(bf16)
        if c == 0:
            c_wv.wait()
        vv = jnp.dot(x, wqkv_v[:, 2 * D:3 * D], preferred_element_type=f32)
        for j in range(CH // 128):
            vvt = vv[128 * j:128 * (j + 1), :].T
            zpad = jnp.zeros((HP - DH, 128), f32)
            parts = []
            for h in range(H):
                parts += [vvt[DH * h:DH * (h + 1), :], zpad]
            vt_s[WIN // 128 + c * (CH // 128) + j] = (
                jnp.concatenate(parts, axis=0).astype(bf16))

    lane = jax.lax.broadcasted_iota(jnp.int32, (QB, 128), 1)

    def hrange(h, t):
        return max(DH * h - 128 * t, 0), min(DH * (h + 1) - 128 * t, 128)

    def attn_body(i, carry):
        r0 = pl.multiple_of(i * QB, QB)
        cc = jax.lax.broadcasted_iota(jnp.int32, (KW, QB), 0)
        rr = jax.lax.broadcasted_iota(jnp.int32, (KW, QB), 1)
        valid = (cc > rr) & (cc <= rr + WIN) & (cc >= WIN - i * QB)
        s_parts = {}
        for t in range(NT):
            qt = q_s[pl.ds(r0, QB), 128 * t:128 * (t + 1)]
            kt = k_s[pl.ds(r0, KW), 128 * t:128 * (t + 1)]
            qm = []
            for h in _UNITS[t]:
                lo, hi = hrange(h, t)
                qm.append(jnp.where((lane >= lo) & (lane < hi), qt, 0.0))
            qs = jnp.concatenate(qm, axis=0).astype(bf16)
            st = jax.lax.dot_general(kt, qs, (((1,), (1,)), ((), ())),
                                     preferred_element_type=f32)
            for u, h in enumerate(_UNITS[t]):
                s_parts.setdefault(h, []).append(st[:, QB * u:QB * (u + 1)])
        for h in range(H):
            s = s_parts[h][0]
            for extra in s_parts[h][1:]:
                s = s + extra
            s = jnp.where(valid, s, NEG)
            mx = jnp.max(s, axis=0, keepdims=True)
            e = jnp.exp2(s - mx)
            l = jnp.sum(e, axis=0, keepdims=True)
            vt = jnp.concatenate(
                [vt_s[i + j, HP * h:HP * (h + 1), :] for j in range(KW // 128)], axis=1)
            ot = jnp.dot(vt, e.astype(bf16), preferred_element_type=f32)
            ot_s[DH * h:DH * (h + 1), :] = (ot * (1.0 / l))[0:DH, :]
        for t in range(NT):
            o_s[pl.ds(r0, QB), 128 * t:128 * (t + 1)] = (
                ot_s[128 * t:128 * (t + 1), :].T.astype(bf16))
        return carry

    jax.lax.fori_loop(0, NQB, attn_body, 0)

    c_wo.wait()
    for c in range(NCH):
        stb_s[c * CH:(c + 1) * CH, :] = jnp.dot(
            o_s[c * CH:(c + 1) * CH, :], wo_v[...], preferred_element_type=f32).astype(bf16)
        oc = pltpu.make_async_copy(stb_s.at[pl.ds(c * CH, CH), :],
                                   out_hbm.at[pl.ds(c * CH, CH), pl.ds(D, D)],
                                   osem.at[c])
        oc.start()
        out_copies.append(oc)

    c_fd.wait()
    c_xa.wait()
    for c in range(NCH):
        xd_s[c * CH:(c + 1) * CH, :] = jnp.dot(
            xa_v[c * CH:(c + 1) * CH, :], fd_v[...], preferred_element_type=f32)

    c_wr.wait()
    c_wi.wait()
    for (w_v, wf_s) in ((wr_v, wfr_s), (wi_v, wfi_s)):
        wt_s[320:DFP, :] = jnp.zeros((DFP - 320, S), f32)
        wt_s[0:DF, :] = w_v[...].astype(f32)
        for lt in range(3):
            wf_s[lt] = wt_s[128 * lt:128 * (lt + 1), :].T

    c_twr.wait()
    c_twi.wait()

    def fwd16_body(rg, carry):
        r8 = pl.multiple_of(rg * 8, 8)
        tw = [(twr_v[pl.ds(N2 * ka + r8, 8), :], twi_v[pl.ds(N2 * ka + r8, 8), :])
              for ka in range(1, N1)]
        for lt in range(DFP // 128):
            x = [(xd_s[pl.ds(N2 * a + r8, 8), 128 * lt:128 * (lt + 1)],
                  xd_s[pl.ds(N2 * a + r8, 8), DFP + 128 * lt:DFP + 128 * (lt + 1)])
                 for a in range(N1)]
            u = _dft16(x, -1)
            for ka in range(N1):
                ur, ui = u[ka]
                if ka > 0:
                    tr, ti = tw[ka - 1]
                    ur, ui = ur * tr - ui * ti, ur * ti + ui * tr
                v16_s[ka, pl.ds(r8, 8), 128 * lt:128 * (lt + 1)] = ur
                v16_s[ka, pl.ds(N2 + r8, 8), 128 * lt:128 * (lt + 1)] = ui
        return carry

    jax.lax.fori_loop(0, N2 // 8, fwd16_body, 0)

    c_ff.wait()
    c_fi.wait()
    for ka in range(N1):
        xx = jnp.dot(ff_v[...], v16_s[ka].astype(bf16), preferred_element_type=f32)
        xr, xi = xx[0:N2, :], xx[N2:2 * N2, :]
        wr = jnp.concatenate(
            [wfr_s[lt, pl.ds(ka, N2, stride=N1), :] for lt in range(3)], axis=1)
        wi = jnp.concatenate(
            [wfi_s[lt, pl.ds(ka, N2, stride=N1), :] for lt in range(3)], axis=1)
        yy = jnp.concatenate([xr * wr - xi * wi, xr * wi + xi * wr], axis=0).astype(bf16)
        v16_s[ka] = jnp.dot(fi_v[...], yy, preferred_element_type=f32)

    def inv16_body(rg, carry):
        r8 = pl.multiple_of(rg * 8, 8)
        tw = [(twr_v[pl.ds(N2 * ka + r8, 8), :], twi_v[pl.ds(N2 * ka + r8, 8), :])
              for ka in range(1, N1)]
        for lt in range(DFP // 128):
            x = []
            for ka in range(N1):
                pr = v16_s[ka, pl.ds(r8, 8), 128 * lt:128 * (lt + 1)]
                pi = v16_s[ka, pl.ds(N2 + r8, 8), 128 * lt:128 * (lt + 1)]
                if ka > 0:
                    tr, ti = tw[ka - 1]
                    pr, pi = pr * tr + pi * ti, pi * tr - pr * ti
                x.append((pr, pi))
            z = _dft16(x, +1)
            for a in range(N1):
                xd_s[pl.ds(N2 * a + r8, 8), 128 * lt:128 * (lt + 1)] = z[a][0]
                xd_s[pl.ds(N2 * a + r8, 8), DFP + 128 * lt:DFP + 128 * (lt + 1)] = z[a][1]
        return carry

    jax.lax.fori_loop(0, N2 // 8, inv16_body, 0)

    c_gd.wait()
    for c in range(NCH):
        sta_s[c * CH:(c + 1) * CH, :] = jnp.dot(
            xd_s[c * CH:(c + 1) * CH, :].astype(bf16), gd_v[...],
            preferred_element_type=f32).astype(bf16)
        oc = pltpu.make_async_copy(sta_s.at[pl.ds(c * CH, CH), :],
                                   out_hbm.at[pl.ds(c * CH, CH), pl.ds(0, D)],
                                   osem.at[NCH + c])
        oc.start()
        out_copies.append(oc)

    for oc in out_copies:
        oc.wait()


@jax.jit
def pallas_concat_heads__spectral_gfnet__sliding_block__prompt_kernel(
    A_x, A_w_r, A_w_i, B_x, B_wqkv, B_wo,
):
    bf16 = jnp.bfloat16
    f32 = jnp.float32
    fd, gd, ff, fi, twr, twi = _make_consts()
    xa = A_x.reshape(S, D)
    xb = B_x.reshape(S, D)
    any_spec = pl.BlockSpec(memory_space=pltpu.MemorySpace.HBM)
    n_in_copies = 14 + NCH - 1
    out = pl.pallas_call(
        _kernel,
        out_shape=jax.ShapeDtypeStruct((S, 2 * D), bf16),
        in_specs=[any_spec] * 12,
        out_specs=any_spec,
        scratch_shapes=[
            pltpu.VMEM((S, D), bf16),
            pltpu.VMEM((D, 3 * D), bf16),
            pltpu.VMEM((D, D), bf16),
            pltpu.VMEM((S, D), bf16),
            pltpu.VMEM((DF, S), bf16),
            pltpu.VMEM((DF, S), bf16),
            pltpu.VMEM((D, 2 * DFP), bf16),
            pltpu.VMEM((2 * DFP, D), bf16),
            pltpu.VMEM((2 * N2, 2 * N2), bf16),
            pltpu.VMEM((2 * N2, 2 * N2), bf16),
            pltpu.VMEM((S, 128), f32),
            pltpu.VMEM((S, 128), f32),
            pltpu.VMEM((S, D), f32),
            pltpu.VMEM((S + WIN, D), bf16),
            pltpu.VMEM(((S + WIN) // 128, H * HP, 128), bf16),
            pltpu.VMEM((D, 128), f32),
            pltpu.VMEM((S, D), bf16),
            pltpu.VMEM((S, 2 * DFP), f32),
            pltpu.VMEM((N1, 2 * N2, DFP), f32),
            pltpu.VMEM((DFP, S), f32),
            pltpu.VMEM((3, S, 128), f32),
            pltpu.VMEM((3, S, 128), f32),
            pltpu.VMEM((S, D), bf16),
            pltpu.VMEM((S, D), bf16),
            pltpu.SemaphoreType.DMA((n_in_copies,)),
            pltpu.SemaphoreType.DMA((2 * NCH,)),
        ],
        compiler_params=pltpu.CompilerParams(
            vmem_limit_bytes=110 * 1024 * 1024),
    )(xb, B_wqkv, B_wo, xa, A_w_r.T, A_w_i.T, fd, gd, ff, fi, twr, twi)
    return out.reshape(1, S, 2 * D)
```

```python
import math

import numpy as np
import jax
import jax.numpy as jnp
from jax.experimental import pallas as pl
from jax.experimental.pallas import tpu as pltpu

S = 2048
D = 640
DF = D // 2 + 1
DFP = 384
H = 32
DH = D // H
WIN = 256
QB = 128
NQB = S // QB
NT = D // 128
KW = WIN + QB
N1 = 16
N2 = 128
CH = 512
NCH = S // CH
CO = 256
NCO = S // CO
NEG = -1e9
WPU = 2 * (CH // 128)
C5 = (math.cos(2 * math.pi / 5), math.cos(4 * math.pi / 5))
S5 = (math.sin(2 * math.pi / 5), math.sin(4 * math.pi / 5))
MIDU = 8
HP = 32

_STRAD = [h for h in range(H) if (DH * h) // 128 != (DH * (h + 1) - 1) // 128]
_UNITS = [[(h, DH * h - 128 * t, DH * (h + 1) - 128 * t) for h in range(H)
           if h not in _STRAD and (DH * h) // 128 == t] for t in range(NT)]
_UNITS.append([(h, DH * e, DH * (e + 1)) for e, h in enumerate(_STRAD)])
DX = D + 128


def _make_consts():
    n2 = np.arange(128)[:, None]
    j = np.arange(128)[None, :]
    m0 = 5 * j
    v0 = (j <= 64).astype(np.float64)
    jj = j % 64
    hi = j >= 64
    m1 = np.where(hi, 4 + 5 * jj, 1 + 5 * jj)
    m2 = np.where(hi, 3 + 5 * jj, 2 + 5 * jj)
    sg = np.where(hi, -1.0, 1.0)

    def cs(m):
        a = 2.0 * np.pi * ((n2 * m) % D) / D
        return np.cos(a), np.sin(a)

    c0, s0 = cs(m0)
    g0f = np.concatenate([c0 * v0, -s0 * v0], axis=1)
    gf = [g0f]
    for mm in (m1, m2):
        c_, s_ = cs(mm)
        gf.append(np.block([[c_, -s_], [sg * s_, sg * c_]]))
    fd = np.concatenate(gf, axis=0)
    sc = 1.0 / (D * S)
    w0 = np.where((j == 0) | (j == 64), 1.0, 2.0) * v0 * sc
    gd0 = np.concatenate([(c0 * w0).T, (-s0 * w0).T], axis=0)
    gd = []
    for mm in (m1, m2):
        c_, s_ = cs(mm)
        gd.append(2.0 * sc * np.block([[c_.T, (sg * s_).T], [-s_.T, (sg * c_).T]]))
    gd = np.concatenate(gd, axis=0)
    kb = np.arange(N2)[:, None]
    b = np.arange(N2)[None, :]
    a2 = 2.0 * np.pi * ((kb * b) % N2) / N2
    cr, sr = np.cos(a2), np.sin(a2)
    ff = np.block([[cr, sr], [-sr, cr]])
    fi = np.block([[cr, -sr], [sr, cr]])
    ka = np.arange(N1)[:, None]
    bb = np.arange(N2)[None, :]
    a3 = (2.0 * np.pi * (ka * bb) / S).reshape(S, 1)
    twr = np.broadcast_to(np.cos(a3), (S, 128))
    twi = np.broadcast_to(-np.sin(a3), (S, 128))
    return (jnp.asarray(fd, jnp.bfloat16), jnp.asarray(gd0, jnp.bfloat16),
            jnp.asarray(gd, jnp.bfloat16),
            jnp.asarray(ff, jnp.bfloat16), jnp.asarray(fi, jnp.bfloat16),
            jnp.asarray(twr, jnp.float32), jnp.asarray(twi, jnp.float32))


def _dft4(x, sign):
    (a0r, a0i), (a1r, a1i), (a2r, a2i), (a3r, a3i) = x
    s0r, s0i = a0r + a2r, a0i + a2i
    d0r, d0i = a0r - a2r, a0i - a2i
    s1r, s1i = a1r + a3r, a1i + a3i
    d1r, d1i = a1r - a3r, a1i - a3i
    if sign < 0:
        x1 = (d0r + d1i, d0i - d1r)
        x3 = (d0r - d1i, d0i + d1r)
    else:
        x1 = (d0r - d1i, d0i + d1r)
        x3 = (d0r + d1i, d0i - d1r)
    return [(s0r + s1r, s0i + s1i), x1, (s0r - s1r, s0i - s1i), x3]


def _cmul_const(xr, xi, e, sign):
    e = e % 16
    if e == 0:
        return xr, xi
    if e == 4:
        return (xi, -xr) if sign < 0 else (-xi, xr)
    ang = sign * 2.0 * math.pi * e / 16.0
    cr, ci = math.cos(ang), math.sin(ang)
    if e in (2, 6):
        r = abs(cr)
        sr = 1.0 if cr > 0 else -1.0
        si = 1.0 if ci > 0 else -1.0
        a = xr * r
        b_ = xi * r
        re = (a if sr > 0 else -a) - (b_ if si > 0 else -b_)
        im = (a if si > 0 else -a) + (b_ if sr > 0 else -b_)
        return re, im
    return xr * cr - xi * ci, xr * ci + xi * cr


def _dft16(x, sign):
    t = [_dft4([x[a0 + 4 * a1] for a1 in range(4)], sign) for a0 in range(4)]
    for a0 in range(1, 4):
        for k1 in range(1, 4):
            t[a0][k1] = _cmul_const(t[a0][k1][0], t[a0][k1][1], a0 * k1, sign)
    out = [None] * 16
    for k1 in range(4):
        u = _dft4([t[a0][k1] for a0 in range(4)], sign)
        for k0 in range(4):
            out[k1 + 4 * k0] = u[k0]
    return out


def _kernel(xb_hbm, wqkv_hbm, wo_hbm, xa_hbm, wr_hbm, wi_hbm,
            fd_hbm, gd0_hbm, gd_hbm, ff_hbm, fi_hbm, twr_hbm, twi_hbm,
            out_hbm,
            xb_v, wqkv_v, wo_v, xa_v, wr_v, wi_v, fd_v, gd0_v, gd_v, ff_v, fi_v, twr_v, twi_v,
            q_s, k_s, vt_s, s_scr0, s_scr1, m_scr0, m_scr1, ot_s, o_s, xd_s, v16_s, wl_s, wfr_s, wfi_s, sta_s, stb_s,
            isem, xbsem, oasem, obsem):
    f32 = jnp.float32
    bf16 = jnp.bfloat16

    n_single = [0]

    def cp(src, dst):
        c = pltpu.make_async_copy(src, dst, isem.at[n_single[0]])
        n_single[0] += 1
        return c

    def xb_copy(c):
        r = pl.multiple_of(c * CH, CH)
        return pltpu.make_async_copy(xb_hbm.at[pl.ds(r, CH), :], xb_v.at[pl.ds(r, CH), :],
                                     xbsem.at[c])

    def outa_copy(c):
        r = pl.multiple_of(c * CH, CH)
        return pltpu.make_async_copy(sta_s.at[pl.ds(r, CH), :],
                                     out_hbm.at[pl.ds(r, CH), pl.ds(0, D)], oasem.at[c])

    def outb_copy(c):
        r = pl.multiple_of(c * CO, CO)
        return pltpu.make_async_copy(stb_s.at[pl.ds(r, CO), :],
                                     out_hbm.at[pl.ds(r, CO), pl.ds(D, D)], obsem.at[c])

    c_wq = cp(wqkv_hbm.at[:, 0:D], wqkv_v.at[:, 0:D])
    c_wk = cp(wqkv_hbm.at[:, D:2 * D], wqkv_v.at[:, D:2 * D])
    c_wv = cp(wqkv_hbm.at[:, 2 * D:3 * D], wqkv_v.at[:, 2 * D:3 * D])
    c_fd = cp(fd_hbm, fd_v)
    c_xa = cp(xa_hbm, xa_v)
    c_wr = cp(wr_hbm, wr_v)
    c_wi = cp(wi_hbm, wi_v)
    c_twr = cp(twr_hbm, twr_v)
    c_twi = cp(twi_hbm, twi_v)
    c_ff = cp(ff_hbm, ff_v)
    c_fi = cp(fi_hbm, fi_v)
    c_wo = cp(wo_hbm, wo_v)
    c_gd = cp(gd_hbm, gd_v)
    c_gd0 = cp(gd0_hbm, gd0_v)

    c_wq.start()
    xb_copy(0).start()

    k_s[0:WIN, :] = jnp.zeros((WIN, DX), bf16)
    for j in range(WIN // 128):
        vt_s[j] = jnp.zeros((H * HP, 128), bf16)
    for u in range(WPU):
        wl_s[u, 320:D, :] = jnp.zeros((D - 320, 128), f32)

    qscale = (DH ** -0.5) * math.log2(math.e)
    c_wq.wait()

    lane_c = jax.lax.broadcasted_iota(jnp.int32, (CH, 128), 1)

    def gather_straddlers(z):
        out = jnp.zeros((CH, 128), f32)
        for e, h in enumerate(_STRAD):
            t = (DH * h) // 128
            lo = DH * h - 128 * t
            n1 = 128 - lo
            p1 = pltpu.roll(z[:, 128 * t:128 * (t + 1)], (DH * e - lo) % 128, 1)
            p2 = pltpu.roll(z[:, 128 * (t + 1):128 * (t + 2)], (DH * e + n1) % 128, 1)
            out = jnp.where((lane_c >= DH * e) & (lane_c < DH * e + n1), p1, out)
            out = jnp.where((lane_c >= DH * e + n1) & (lane_c < DH * (e + 1)), p2, out)
        return out

    def qkv_body(c, carry):
        xb_copy(c).wait()

        @pl.when(c == 0)
        def _():
            c_wk.start()
            c_wv.start()

        @pl.when(c + 1 < NCH)
        def _():
            xb_copy(jnp.minimum(c + 1, NCH - 1)).start()

        @pl.when(c == 1)
        def _():
            c_fd.start()
            c_xa.start()
            c_wr.start()
            c_wi.start()

        @pl.when(c == 2)
        def _():
            c_twr.start()
            c_twi.start()
            c_ff.start()
            c_fi.start()

        @pl.when(c == 3)
        def _():
            c_wo.start()
            c_gd.start()
            c_gd0.start()

        r = pl.multiple_of(c * CH, CH)
        x = xb_v[pl.ds(r, CH), :]
        qq = qscale * jnp.dot(x, wqkv_v[:, 0:D], preferred_element_type=f32)
        q_s[pl.ds(r, CH), 0:D] = qq
        q_s[pl.ds(r, CH), D:DX] = gather_straddlers(qq)

        @pl.when(c == 0)
        def _():
            c_wk.wait()
            c_wv.wait()

        kk = jnp.dot(x, wqkv_v[:, D:2 * D], preferred_element_type=f32)
        k_s[pl.ds(WIN + r, CH), 0:D] = kk.astype(bf16)
        k_s[pl.ds(WIN + r, CH), D:DX] = gather_straddlers(kk).astype(bf16)
        vv = jnp.dot(x, wqkv_v[:, 2 * D:3 * D], preferred_element_type=f32)
        for j in range(CH // 128):
            vvt = vv[128 * j:128 * (j + 1), :].T
            zpad = jnp.zeros((HP - DH, 128), f32)
            parts = []
            for h in range(H):
                parts += [vvt[DH * h:DH * (h + 1), :], zpad]
            vt_s[WIN // 128 + c * (CH // 128) + j] = (
                jnp.concatenate(parts, axis=0).astype(bf16))
        return carry

    jax.lax.fori_loop(0, NCH, qkv_body, 0)

    c_fd.wait()
    c_xa.wait()
    c_wr.wait()
    c_wi.wait()

    def rfft_body(c, carry):
        r = pl.multiple_of(c * CH, CH)
        xt = [xa_v[pl.ds(r, CH), 128 * t:128 * (t + 1)].astype(f32) for t in range(5)]
        t1, t2 = xt[1] + xt[4], xt[2] + xt[3]
        t3, t4 = xt[1] - xt[4], xt[2] - xt[3]
        a0 = (xt[0] + t1 + t2).astype(bf16)
        a1 = jnp.concatenate([xt[0] + C5[0] * t1 + C5[1] * t2,
                              -(S5[0] * t3 + S5[1] * t4)], axis=1).astype(bf16)
        a2 = jnp.concatenate([xt[0] + C5[1] * t1 + C5[0] * t2,
                              S5[0] * t4 - S5[1] * t3], axis=1).astype(bf16)
        for t, (aa, lo, hi_) in enumerate(((a0, 0, 128), (a1, 128, 384), (a2, 384, 640))):
            tt = jnp.dot(aa, fd_v[lo:hi_, :], preferred_element_type=f32)
            xd_s[pl.ds(r, CH), 128 * t:128 * (t + 1)] = tt[:, 0:128]
            xd_s[pl.ds(r, CH), DFP + 128 * t:DFP + 128 * (t + 1)] = tt[:, 128:256]
        u = 0
        for jj in range(CH // 128):
            cl = pl.multiple_of(r + jj * 128, 128)
            for (w_v, wf_s) in ((wr_v, wfr_s), (wi_v, wfi_s)):
                wl_s[u, 0:DF, :] = w_v[:, pl.ds(cl, 128)].astype(f32)
                blocks = (
                    wl_s[u, pl.ds(0, 128, stride=5), :],
                    jnp.concatenate([wl_s[u, pl.ds(1, 64, stride=5), :],
                                     wl_s[u, pl.ds(4, 64, stride=5), :]], axis=0),
                    jnp.concatenate([wl_s[u, pl.ds(2, 64, stride=5), :],
                                     wl_s[u, pl.ds(3, 64, stride=5), :]], axis=0))
                for lt in range(3):
                    wf_s[lt, pl.ds(cl, 128), :] = blocks[lt].astype(bf16).T.astype(f32)
                u += 1
        return carry

    jax.lax.fori_loop(0, NCH, rfft_body, 0)

    c_twr.wait()
    c_twi.wait()

    def fwd16(rg):
        r8 = pl.multiple_of(rg * 8, 8)
        tw = [(twr_v[pl.ds(N2 * ka + r8, 8), :], twi_v[pl.ds(N2 * ka + r8, 8), :])
              for ka in range(1, N1)]
        for lt in range(DFP // 128):
            x = [(xd_s[pl.ds(N2 * a + r8, 8), 128 * lt:128 * (lt + 1)],
                  xd_s[pl.ds(N2 * a + r8, 8), DFP + 128 * lt:DFP + 128 * (lt + 1)])
                 for a in range(N1)]
            u = _dft16(x, -1)
            for ka in range(N1):
                ur, ui = u[ka]
                if ka > 0:
                    tr, ti = tw[ka - 1]
                    ur, ui = ur * tr - ui * ti, ur * ti + ui * tr
                v16_s[ka, pl.ds(r8, 8), 128 * lt:128 * (lt + 1)] = ur
                v16_s[ka, pl.ds(N2 + r8, 8), 128 * lt:128 * (lt + 1)] = ui

    def inv16(rg):
        r8 = pl.multiple_of(rg * 8, 8)
        tw = [(twr_v[pl.ds(N2 * ka + r8, 8), :], twi_v[pl.ds(N2 * ka + r8, 8), :])
              for ka in range(1, N1)]
        for lt in range(DFP // 128):
            x = []
            for ka in range(N1):
                pr = v16_s[ka, pl.ds(r8, 8), 128 * lt:128 * (lt + 1)]
                pi = v16_s[ka, pl.ds(N2 + r8, 8), 128 * lt:128 * (lt + 1)]
                if ka > 0:
                    tr, ti = tw[ka - 1]
                    pr, pi = pr * tr + pi * ti, pi * tr - pr * ti
                x.append((pr, pi))
            z = _dft16(x, +1)
            for a in range(N1):
                xd_s[pl.ds(N2 * a + r8, 8), 128 * lt:128 * (lt + 1)] = z[a][0]
                xd_s[pl.ds(N2 * a + r8, 8), DFP + 128 * lt:DFP + 128 * (lt + 1)] = z[a][1]

    lane = jax.lax.broadcasted_iota(jnp.int32, (QB, 128), 1)

    s_bufs = (s_scr0, s_scr1)
    m_bufs = (m_scr0, m_scr1)

    def attn_scores(i, slot):
        r0 = pl.multiple_of(i * QB, QB)
        cc = jax.lax.broadcasted_iota(jnp.int32, (KW, QB), 0)
        rr = jax.lax.broadcasted_iota(jnp.int32, (KW, QB), 1)
        valid = (cc > rr) & (cc <= rr + WIN) & (cc >= WIN - i * QB)
        for t in range(NT + 1):
            qt = q_s[pl.ds(r0, QB), 128 * t:128 * (t + 1)]
            kt = k_s[pl.ds(r0, KW), 128 * t:128 * (t + 1)]
            qs = jnp.concatenate(
                [jnp.where((lane >= lo) & (lane < hi), qt, 0.0) for (_, lo, hi) in _UNITS[t]],
                axis=0).astype(bf16)
            st = jax.lax.dot_general(kt, qs, (((1,), (1,)), ((), ())),
                                     preferred_element_type=f32)
            for u, (h, _, _) in enumerate(_UNITS[t]):
                sh = jnp.where(valid, st[:, QB * u:QB * (u + 1)], NEG)
                s_bufs[slot][h] = sh
                m_bufs[slot][h] = jnp.broadcast_to(
                    jnp.max(sh, axis=0, keepdims=True), (8, QB))

    def attn_finish(i, slot):
        r0 = pl.multiple_of(i * QB, QB)
        for h in range(H):
            e = jnp.exp2(s_bufs[slot][h] - m_bufs[slot][h, 0:1, :])
            l = jnp.sum(e, axis=0, keepdims=True)
            vt = jnp.concatenate(
                [vt_s[i + j, HP * h:HP * (h + 1), :] for j in range(KW // 128)], axis=1)
            ot = jnp.dot(vt, e.astype(bf16), preferred_element_type=f32)
            ot_s[DH * h:DH * (h + 1), :] = (ot * (1.0 / l))[0:DH, :]
        for t in range(NT):
            o_s[pl.ds(r0, QB), 128 * t:128 * (t + 1)] = (
                ot_s[128 * t:128 * (t + 1), :].T.astype(bf16))

    attn_scores(0, 0)

    def body1(j, carry):
        attn_scores(2 * j + 1, 1)
        attn_finish(2 * j, 0)
        fwd16(4 * j)
        fwd16(4 * j + 1)
        attn_scores(2 * j + 2, 0)
        attn_finish(2 * j + 1, 1)
        fwd16(4 * j + 2)
        fwd16(4 * j + 3)
        return carry

    jax.lax.fori_loop(0, NQB // 4, body1, 0)

    c_ff.wait()
    c_fi.wait()

    def mid_body(g, carry):
        for kk in range(MIDU):
            ka = g * MIDU + kk
            xx = jnp.dot(ff_v[...], v16_s[ka].astype(bf16), preferred_element_type=f32)
            xr, xi = xx[0:N2, :], xx[N2:2 * N2, :]
            wr = jnp.concatenate(
                [wfr_s[lt, pl.ds(ka, N2, stride=N1), :] for lt in range(3)], axis=1)
            wi = jnp.concatenate(
                [wfi_s[lt, pl.ds(ka, N2, stride=N1), :] for lt in range(3)], axis=1)
            yy = jnp.concatenate([xr * wr - xi * wi, xr * wi + xi * wr],
                                 axis=0).astype(bf16)
            v16_s[ka] = jnp.dot(fi_v[...], yy, preferred_element_type=f32)
        return carry

    jax.lax.fori_loop(0, N1 // MIDU, mid_body, 0)

    def body2(j, carry, last=False):
        ib = 2 * j + NQB // 2
        attn_scores(ib + 1, 1)
        attn_finish(ib, 0)
        inv16(4 * j)
        inv16(4 * j + 1)
        if not last:
            attn_scores(ib + 2, 0)
        attn_finish(ib + 1, 1)
        inv16(4 * j + 2)
        inv16(4 * j + 3)
        return carry

    jax.lax.fori_loop(0, NQB // 4 - 1, body2, 0)
    body2(NQB // 4 - 1, 0, last=True)

    c_gd.wait()
    c_gd0.wait()

    def irfft_body(c, carry):
        r = pl.multiple_of(c * CH, CH)
        zz = [jnp.concatenate(
            [xd_s[pl.ds(r, CH), 128 * t:128 * (t + 1)],
             xd_s[pl.ds(r, CH), DFP + 128 * t:DFP + 128 * (t + 1)]], axis=1).astype(bf16)
            for t in range(3)]
        c0 = jnp.dot(zz[0], gd0_v[...], preferred_element_type=f32)
        e1 = jnp.dot(zz[1], gd_v[0:256, :], preferred_element_type=f32)
        e2 = jnp.dot(zz[2], gd_v[256:512, :], preferred_element_type=f32)
        e1r, e1i, e2r, e2i = e1[:, 0:128], e1[:, 128:256], e2[:, 0:128], e2[:, 128:256]
        p1 = c0 + C5[0] * e1r + C5[1] * e2r
        q1 = S5[0] * e1i + S5[1] * e2i
        p2 = c0 + C5[1] * e1r + C5[0] * e2r
        q2 = S5[1] * e1i - S5[0] * e2i
        ys = (c0 + e1r + e2r, p1 - q1, p2 - q2, p2 + q2, p1 + q1)
        for t in range(5):
            sta_s[pl.ds(r, CH), 128 * t:128 * (t + 1)] = ys[t].astype(bf16)
        outa_copy(c).start()
        return carry

    jax.lax.fori_loop(0, NCH, irfft_body, 0)

    c_wo.wait()

    def oproj_body(c, carry):
        r = pl.multiple_of(c * CO, CO)
        stb_s[pl.ds(r, CO), :] = jnp.dot(
            o_s[pl.ds(r, CO), :], wo_v[...], preferred_element_type=f32).astype(bf16)
        outb_copy(c).start()
        return carry

    jax.lax.fori_loop(0, NCO, oproj_body, 0)

    for c in range(NCO):
        outb_copy(c).wait()
    for c in range(NCH):
        outa_copy(c).wait()


@jax.jit
def pallas_concat_heads__spectral_gfnet__sliding_block__prompt_kernel(
    A_x, A_w_r, A_w_i, B_x, B_wqkv, B_wo,
):
    bf16 = jnp.bfloat16
    f32 = jnp.float32
    fd, gd0, gd, ff, fi, twr, twi = _make_consts()
    xa = A_x.reshape(S, D)
    xb = B_x.reshape(S, D)
    any_spec = pl.BlockSpec(memory_space=pltpu.MemorySpace.HBM)
    out = pl.pallas_call(
        _kernel,
        out_shape=jax.ShapeDtypeStruct((S, 2 * D), bf16),
        in_specs=[any_spec] * 13,
        out_specs=any_spec,
        scratch_shapes=[
            pltpu.VMEM((S, D), bf16),
            pltpu.VMEM((D, 3 * D), bf16),
            pltpu.VMEM((D, D), bf16),
            pltpu.VMEM((S, D), bf16),
            pltpu.VMEM((DF, S), bf16),
            pltpu.VMEM((DF, S), bf16),
            pltpu.VMEM((D, 256), bf16),
            pltpu.VMEM((256, 128), bf16),
            pltpu.VMEM((512, 256), bf16),
            pltpu.VMEM((2 * N2, 2 * N2), bf16),
            pltpu.VMEM((2 * N2, 2 * N2), bf16),
            pltpu.VMEM((S, 128), f32),
            pltpu.VMEM((S, 128), f32),
            pltpu.VMEM((S, DX), f32),
            pltpu.VMEM((S + WIN, DX), bf16),
            pltpu.VMEM(((S + WIN) // 128, H * HP, 128), bf16),
            pltpu.VMEM((H, KW, QB), f32),
            pltpu.VMEM((H, KW, QB), f32),
            pltpu.VMEM((H, 8, QB), f32),
            pltpu.VMEM((H, 8, QB), f32),
            pltpu.VMEM((D, 128), f32),
            pltpu.VMEM((S, D), bf16),
            pltpu.VMEM((S, 2 * DFP), f32),
            pltpu.VMEM((N1, 2 * N2, DFP), f32),
            pltpu.VMEM((WPU, D, 128), f32),
            pltpu.VMEM((3, S, 128), f32),
            pltpu.VMEM((3, S, 128), f32),
            pltpu.VMEM((S, D), bf16),
            pltpu.VMEM((S, D), bf16),
            pltpu.SemaphoreType.DMA((14,)),
            pltpu.SemaphoreType.DMA((NCH,)),
            pltpu.SemaphoreType.DMA((NCH,)),
            pltpu.SemaphoreType.DMA((NCO,)),
        ],
        compiler_params=pltpu.CompilerParams(
            vmem_limit_bytes=110 * 1024 * 1024),
    )(xb, B_wqkv, B_wo, xa, A_w_r.T, A_w_i.T, fd, gd0, gd, ff, fi, twr, twi)
    return out.reshape(1, S, 2 * D)
```

```python
import math

import numpy as np
import jax
import jax.numpy as jnp
from jax.experimental import pallas as pl
from jax.experimental.pallas import tpu as pltpu

S = 2048
D = 640
DF = D // 2 + 1
DFP = 384
H = 32
DH = D // H
WIN = 256
QB = 128
NQB = S // QB
NT = D // 128
KW = WIN + QB
N1 = 16
N2 = 128
CH = 512
NCH = S // CH
CO = 256
NCO = S // CO
NEG = -1e9
WPU = 2 * (CH // 128)
C5 = (math.cos(2 * math.pi / 5), math.cos(4 * math.pi / 5))
S5 = (math.sin(2 * math.pi / 5), math.sin(4 * math.pi / 5))
MIDU = 8
HP = 32

_STRAD = [h for h in range(H) if (DH * h) // 128 != (DH * (h + 1) - 1) // 128]
_UNITS = [[(h, DH * h - 128 * t, DH * (h + 1) - 128 * t) for h in range(H)
           if h not in _STRAD and (DH * h) // 128 == t] for t in range(NT)]
_UNITS.append([(h, DH * e, DH * (e + 1)) for e, h in enumerate(_STRAD)])
DX = D + 128


def _make_consts():
    n2 = np.arange(128)[:, None]
    j = np.arange(128)[None, :]
    m0 = 5 * j
    v0 = (j <= 64).astype(np.float64)
    jj = j % 64
    hi = j >= 64
    m1 = np.where(hi, 4 + 5 * jj, 1 + 5 * jj)
    m2 = np.where(hi, 3 + 5 * jj, 2 + 5 * jj)
    sg = np.where(hi, -1.0, 1.0)

    def cs(m):
        a = 2.0 * np.pi * ((n2 * m) % D) / D
        return np.cos(a), np.sin(a)

    c0, s0 = cs(m0)
    g0f = np.concatenate([c0 * v0, -s0 * v0], axis=1)
    gf = [g0f]
    for mm in (m1, m2):
        c_, s_ = cs(mm)
        gf.append(np.block([[c_, -s_], [sg * s_, sg * c_]]))
    fd = np.concatenate(gf, axis=0)
    sc = 1.0 / (D * S)
    w0 = np.where((j == 0) | (j == 64), 1.0, 2.0) * v0 * sc
    gd0 = np.concatenate([(c0 * w0).T, (-s0 * w0).T], axis=0)
    gd = []
    for mm in (m1, m2):
        c_, s_ = cs(mm)
        gd.append(2.0 * sc * np.block([[c_.T, (sg * s_).T], [-s_.T, (sg * c_).T]]))
    gd = np.concatenate(gd, axis=0)
    kb = np.arange(N2)[:, None]
    b = np.arange(N2)[None, :]
    a2 = 2.0 * np.pi * ((kb * b) % N2) / N2
    cr, sr = np.cos(a2), np.sin(a2)
    ff = np.block([[cr, sr], [-sr, cr]])
    fi = np.block([[cr, -sr], [sr, cr]])
    ka = np.arange(N1)[:, None]
    bb = np.arange(N2)[None, :]
    a3 = (2.0 * np.pi * (ka * bb) / S).reshape(S, 1)
    twr = np.broadcast_to(np.cos(a3), (S, 128))
    twi = np.broadcast_to(-np.sin(a3), (S, 128))
    return (jnp.asarray(fd, jnp.bfloat16), jnp.asarray(gd0, jnp.bfloat16),
            jnp.asarray(gd, jnp.bfloat16),
            jnp.asarray(ff, jnp.bfloat16), jnp.asarray(fi, jnp.bfloat16),
            jnp.asarray(twr, jnp.float32), jnp.asarray(twi, jnp.float32))


def _dft4(x, sign):
    (a0r, a0i), (a1r, a1i), (a2r, a2i), (a3r, a3i) = x
    s0r, s0i = a0r + a2r, a0i + a2i
    d0r, d0i = a0r - a2r, a0i - a2i
    s1r, s1i = a1r + a3r, a1i + a3i
    d1r, d1i = a1r - a3r, a1i - a3i
    if sign < 0:
        x1 = (d0r + d1i, d0i - d1r)
        x3 = (d0r - d1i, d0i + d1r)
    else:
        x1 = (d0r - d1i, d0i + d1r)
        x3 = (d0r + d1i, d0i - d1r)
    return [(s0r + s1r, s0i + s1i), x1, (s0r - s1r, s0i - s1i), x3]


def _cmul_const(xr, xi, e, sign):
    e = e % 16
    if e == 0:
        return xr, xi
    if e == 4:
        return (xi, -xr) if sign < 0 else (-xi, xr)
    ang = sign * 2.0 * math.pi * e / 16.0
    cr, ci = math.cos(ang), math.sin(ang)
    if e in (2, 6):
        r = abs(cr)
        sr = 1.0 if cr > 0 else -1.0
        si = 1.0 if ci > 0 else -1.0
        a = xr * r
        b_ = xi * r
        re = (a if sr > 0 else -a) - (b_ if si > 0 else -b_)
        im = (a if si > 0 else -a) + (b_ if sr > 0 else -b_)
        return re, im
    return xr * cr - xi * ci, xr * ci + xi * cr


def _dft16(x, sign):
    t = [_dft4([x[a0 + 4 * a1] for a1 in range(4)], sign) for a0 in range(4)]
    for a0 in range(1, 4):
        for k1 in range(1, 4):
            t[a0][k1] = _cmul_const(t[a0][k1][0], t[a0][k1][1], a0 * k1, sign)
    out = [None] * 16
    for k1 in range(4):
        u = _dft4([t[a0][k1] for a0 in range(4)], sign)
        for k0 in range(4):
            out[k1 + 4 * k0] = u[k0]
    return out


def _kernel(xb_hbm, wqkv_hbm, wo_hbm, xa_hbm, wr_hbm, wi_hbm,
            fd_hbm, gd0_hbm, gd_hbm, ff_hbm, fi_hbm, twr_hbm, twi_hbm,
            out_hbm,
            xb_v, wqkv_v, wo_v, xa_v, wr_v, wi_v, fd_v, gd0_v, gd_v, ff_v, fi_v, twr_v, twi_v,
            q_s, k_s, vt_s, s_scr0, s_scr1, m_scr0, m_scr1, ot_s, o_s, xd_s, v16_s, wl_s, wfr_s, wfi_s, sta_s, stb_s,
            isem, xbsem, oasem, obsem):
    f32 = jnp.float32
    bf16 = jnp.bfloat16

    n_single = [0]

    def cp(src, dst):
        c = pltpu.make_async_copy(src, dst, isem.at[n_single[0]])
        n_single[0] += 1
        return c

    def xb_copy(c):
        r = pl.multiple_of(c * CH, CH)
        return pltpu.make_async_copy(xb_hbm.at[pl.ds(r, CH), :], xb_v.at[pl.ds(r, CH), :],
                                     xbsem.at[c])

    def outa_copy(c):
        r = pl.multiple_of(c * CH, CH)
        return pltpu.make_async_copy(sta_s.at[pl.ds(r, CH), :],
                                     out_hbm.at[pl.ds(r, CH), pl.ds(0, D)], oasem.at[c])

    def outb_copy(c):
        r = pl.multiple_of(c * CO, CO)
        return pltpu.make_async_copy(stb_s.at[pl.ds(r, CO), :],
                                     out_hbm.at[pl.ds(r, CO), pl.ds(D, D)], obsem.at[c])

    c_wq = cp(wqkv_hbm.at[:, 0:D], wqkv_v.at[:, 0:D])
    c_wk = cp(wqkv_hbm.at[:, D:2 * D], wqkv_v.at[:, D:2 * D])
    c_wv = cp(wqkv_hbm.at[:, 2 * D:3 * D], wqkv_v.at[:, 2 * D:3 * D])
    c_fd = cp(fd_hbm, fd_v)
    c_xa = cp(xa_hbm, xa_v)
    c_wr = cp(wr_hbm, wr_v)
    c_wi = cp(wi_hbm, wi_v)
    c_twr = cp(twr_hbm, twr_v)
    c_twi = cp(twi_hbm, twi_v)
    c_ff = cp(ff_hbm, ff_v)
    c_fi = cp(fi_hbm, fi_v)
    c_wo = cp(wo_hbm, wo_v)
    c_gd = cp(gd_hbm, gd_v)
    c_gd0 = cp(gd0_hbm, gd0_v)

    c_wq.start()
    xb_copy(0).start()

    k_s[0:WIN, :] = jnp.zeros((WIN, DX), bf16)
    for j in range(WIN // 128):
        vt_s[j] = jnp.zeros((H * HP, 128), bf16)
    for u in range(WPU):
        wl_s[u, 320:D, :] = jnp.zeros((D - 320, 128), f32)

    qscale = (DH ** -0.5) * math.log2(math.e)
    c_wq.wait()

    lane_c = jax.lax.broadcasted_iota(jnp.int32, (CH, 128), 1)

    def gather_straddlers(z):
        out = jnp.zeros((CH, 128), f32)
        for e, h in enumerate(_STRAD):
            t = (DH * h) // 128
            lo = DH * h - 128 * t
            n1 = 128 - lo
            p1 = pltpu.roll(z[:, 128 * t:128 * (t + 1)], (DH * e - lo) % 128, 1)
            p2 = pltpu.roll(z[:, 128 * (t + 1):128 * (t + 2)], (DH * e + n1) % 128, 1)
            out = jnp.where((lane_c >= DH * e) & (lane_c < DH * e + n1), p1, out)
            out = jnp.where((lane_c >= DH * e + n1) & (lane_c < DH * (e + 1)), p2, out)
        return out

    def q_body(c, carry):
        xb_copy(c).wait()

        @pl.when(c + 1 < NCH)
        def _():
            xb_copy(jnp.minimum(c + 1, NCH - 1)).start()

        @pl.when(c == 1)
        def _():
            c_wk.start()

        @pl.when(c == 3)
        def _():
            c_wv.start()
            c_fd.start()

        r = pl.multiple_of(c * CH, CH)
        qq = qscale * jnp.dot(xb_v[pl.ds(r, CH), :], wqkv_v[:, 0:D],
                              preferred_element_type=f32)
        q_s[pl.ds(r, CH), 0:D] = qq
        q_s[pl.ds(r, CH), D:DX] = gather_straddlers(qq)
        return carry

    jax.lax.fori_loop(0, NCH, q_body, 0)
    c_wk.wait()

    def k_body(c, carry):
        @pl.when(c == 0)
        def _():
            c_xa.start()

        @pl.when(c == 1)
        def _():
            c_wr.start()
            c_wi.start()

        r = pl.multiple_of(c * CH, CH)
        kk = jnp.dot(xb_v[pl.ds(r, CH), :], wqkv_v[:, D:2 * D], preferred_element_type=f32)
        k_s[pl.ds(WIN + r, CH), 0:D] = kk.astype(bf16)
        k_s[pl.ds(WIN + r, CH), D:DX] = gather_straddlers(kk).astype(bf16)
        return carry

    jax.lax.fori_loop(0, NCH, k_body, 0)
    c_wv.wait()
    c_fd.wait()
    c_xa.wait()
    c_wr.wait()
    c_wi.wait()

    def rfft_body(c, carry):
        r = pl.multiple_of(c * CH, CH)
        xt = [xa_v[pl.ds(r, CH), 128 * t:128 * (t + 1)].astype(f32) for t in range(5)]
        t1, t2 = xt[1] + xt[4], xt[2] + xt[3]
        t3, t4 = xt[1] - xt[4], xt[2] - xt[3]
        a0 = (xt[0] + t1 + t2).astype(bf16)
        a1 = jnp.concatenate([xt[0] + C5[0] * t1 + C5[1] * t2,
                              -(S5[0] * t3 + S5[1] * t4)], axis=1).astype(bf16)
        a2 = jnp.concatenate([xt[0] + C5[1] * t1 + C5[0] * t2,
                              S5[0] * t4 - S5[1] * t3], axis=1).astype(bf16)
        for t, (aa, lo, hi_) in enumerate(((a0, 0, 128), (a1, 128, 384), (a2, 384, 640))):
            tt = jnp.dot(aa, fd_v[lo:hi_, :], preferred_element_type=f32)
            xd_s[pl.ds(r, CH), 128 * t:128 * (t + 1)] = tt[:, 0:128]
            xd_s[pl.ds(r, CH), DFP + 128 * t:DFP + 128 * (t + 1)] = tt[:, 128:256]
        u = 0
        for jj in range(CH // 128):
            cl = pl.multiple_of(r + jj * 128, 128)
            for (w_v, wf_s) in ((wr_v, wfr_s), (wi_v, wfi_s)):
                wl_s[u, 0:DF, :] = w_v[:, pl.ds(cl, 128)].astype(f32)
                blocks = (
                    wl_s[u, pl.ds(0, 128, stride=5), :],
                    jnp.concatenate([wl_s[u, pl.ds(1, 64, stride=5), :],
                                     wl_s[u, pl.ds(4, 64, stride=5), :]], axis=0),
                    jnp.concatenate([wl_s[u, pl.ds(2, 64, stride=5), :],
                                     wl_s[u, pl.ds(3, 64, stride=5), :]], axis=0))
                for lt in range(3):
                    wf_s[lt, pl.ds(cl, 128), :] = blocks[lt].astype(bf16).T.astype(f32)
                u += 1
        return carry

    def v_body(c, carry):
        @pl.when(c == 1)
        def _():
            c_twr.start()
            c_twi.start()

        @pl.when(c == 2)
        def _():
            c_ff.start()
            c_fi.start()
            c_wo.start()

        @pl.when(c == 3)
        def _():
            c_gd.start()
            c_gd0.start()

        r = pl.multiple_of(c * CH, CH)
        vv = jnp.dot(xb_v[pl.ds(r, CH), :], wqkv_v[:, 2 * D:3 * D],
                     preferred_element_type=f32)
        for j in range(CH // 128):
            vvt = vv[128 * j:128 * (j + 1), :].T
            zpad = jnp.zeros((HP - DH, 128), f32)
            parts = []
            for h in range(H):
                parts += [vvt[DH * h:DH * (h + 1), :], zpad]
            vt_s[WIN // 128 + c * (CH // 128) + j] = (
                jnp.concatenate(parts, axis=0).astype(bf16))
        rfft_body(c, carry)
        return carry

    jax.lax.fori_loop(0, NCH, v_body, 0)

    c_twr.wait()
    c_twi.wait()

    def fwd16(rg):
        r8 = pl.multiple_of(rg * 8, 8)
        tw = [(twr_v[pl.ds(N2 * ka + r8, 8), :], twi_v[pl.ds(N2 * ka + r8, 8), :])
              for ka in range(1, N1)]
        for lt in range(DFP // 128):
            x = [(xd_s[pl.ds(N2 * a + r8, 8), 128 * lt:128 * (lt + 1)],
                  xd_s[pl.ds(N2 * a + r8, 8), DFP + 128 * lt:DFP + 128 * (lt + 1)])
                 for a in range(N1)]
            u = _dft16(x, -1)
            for ka in range(N1):
                ur, ui = u[ka]
                if ka > 0:
                    tr, ti = tw[ka - 1]
                    ur, ui = ur * tr - ui * ti, ur * ti + ui * tr
                v16_s[ka, pl.ds(r8, 8), 128 * lt:128 * (lt + 1)] = ur
                v16_s[ka, pl.ds(N2 + r8, 8), 128 * lt:128 * (lt + 1)] = ui

    def inv16(rg):
        r8 = pl.multiple_of(rg * 8, 8)
        tw = [(twr_v[pl.ds(N2 * ka + r8, 8), :], twi_v[pl.ds(N2 * ka + r8, 8), :])
              for ka in range(1, N1)]
        for lt in range(DFP // 128):
            x = []
            for ka in range(N1):
                pr = v16_s[ka, pl.ds(r8, 8), 128 * lt:128 * (lt + 1)]
                pi = v16_s[ka, pl.ds(N2 + r8, 8), 128 * lt:128 * (lt + 1)]
                if ka > 0:
                    tr, ti = tw[ka - 1]
                    pr, pi = pr * tr + pi * ti, pi * tr - pr * ti
                x.append((pr, pi))
            z = _dft16(x, +1)
            for a in range(N1):
                xd_s[pl.ds(N2 * a + r8, 8), 128 * lt:128 * (lt + 1)] = z[a][0]
                xd_s[pl.ds(N2 * a + r8, 8), DFP + 128 * lt:DFP + 128 * (lt + 1)] = z[a][1]

    lane = jax.lax.broadcasted_iota(jnp.int32, (QB, 128), 1)

    s_bufs = (s_scr0, s_scr1)
    m_bufs = (m_scr0, m_scr1)

    def attn_scores(i, slot):
        r0 = pl.multiple_of(i * QB, QB)
        cc = jax.lax.broadcasted_iota(jnp.int32, (KW, QB), 0)
        rr = jax.lax.broadcasted_iota(jnp.int32, (KW, QB), 1)
        valid = (cc > rr) & (cc <= rr + WIN) & (cc >= WIN - i * QB)
        for t in range(NT + 1):
            qt = q_s[pl.ds(r0, QB), 128 * t:128 * (t + 1)]
            kt = k_s[pl.ds(r0, KW), 128 * t:128 * (t + 1)]
            qs = jnp.concatenate(
                [jnp.where((lane >= lo) & (lane < hi), qt, 0.0) for (_, lo, hi) in _UNITS[t]],
                axis=0).astype(bf16)
            st = jax.lax.dot_general(kt, qs, (((1,), (1,)), ((), ())),
                                     preferred_element_type=f32)
            for u, (h, _, _) in enumerate(_UNITS[t]):
                sh = jnp.where(valid, st[:, QB * u:QB * (u + 1)], NEG)
                s_bufs[slot][h] = sh
                m_bufs[slot][h] = jnp.broadcast_to(
                    jnp.max(sh, axis=0, keepdims=True), (8, QB))

    def attn_finish(i, slot):
        r0 = pl.multiple_of(i * QB, QB)
        for h in range(H):
            e = jnp.exp2(s_bufs[slot][h] - m_bufs[slot][h, 0:1, :])
            l = jnp.sum(e, axis=0, keepdims=True)
            vt = jnp.concatenate(
                [vt_s[i + j, HP * h:HP * (h + 1), :] for j in range(KW // 128)], axis=1)
            ot = jnp.dot(vt, e.astype(bf16), preferred_element_type=f32)
            ot_s[DH * h:DH * (h + 1), :] = (ot * (1.0 / l))[0:DH, :]
        for t in range(NT):
            o_s[pl.ds(r0, QB), 128 * t:128 * (t + 1)] = (
                ot_s[128 * t:128 * (t + 1), :].T.astype(bf16))

    attn_scores(0, 0)

    def body1(j, carry):
        attn_scores(2 * j + 1, 1)
        attn_finish(2 * j, 0)
        fwd16(4 * j)
        fwd16(4 * j + 1)
        attn_scores(2 * j + 2, 0)
        attn_finish(2 * j + 1, 1)
        fwd16(4 * j + 2)
        fwd16(4 * j + 3)
        return carry

    jax.lax.fori_loop(0, NQB // 4, body1, 0)

    c_ff.wait()
    c_fi.wait()

    def mid_body(g, carry):
        for kk in range(MIDU):
            ka = g * MIDU + kk
            xx = jnp.dot(ff_v[...], v16_s[ka].astype(bf16), preferred_element_type=f32)
            xr, xi = xx[0:N2, :], xx[N2:2 * N2, :]
            wr = jnp.concatenate(
                [wfr_s[lt, pl.ds(ka, N2, stride=N1), :] for lt in range(3)], axis=1)
            wi = jnp.concatenate(
                [wfi_s[lt, pl.ds(ka, N2, stride=N1), :] for lt in range(3)], axis=1)
            yy = jnp.concatenate([xr * wr - xi * wi, xr * wi + xi * wr],
                                 axis=0).astype(bf16)
            v16_s[ka] = jnp.dot(fi_v[...], yy, preferred_element_type=f32)
        return carry

    jax.lax.fori_loop(0, N1 // MIDU, mid_body, 0)

    def body2(j, carry, last=False):
        ib = 2 * j + NQB // 2
        attn_scores(ib + 1, 1)
        attn_finish(ib, 0)
        inv16(4 * j)
        inv16(4 * j + 1)
        if not last:
            attn_scores(ib + 2, 0)
        attn_finish(ib + 1, 1)
        inv16(4 * j + 2)
        inv16(4 * j + 3)
        return carry

    jax.lax.fori_loop(0, NQB // 4 - 1, body2, 0)
    body2(NQB // 4 - 1, 0, last=True)

    c_gd.wait()
    c_gd0.wait()

    def irfft_body(c, carry):
        r = pl.multiple_of(c * CH, CH)
        zz = [jnp.concatenate(
            [xd_s[pl.ds(r, CH), 128 * t:128 * (t + 1)],
             xd_s[pl.ds(r, CH), DFP + 128 * t:DFP + 128 * (t + 1)]], axis=1).astype(bf16)
            for t in range(3)]
        c0 = jnp.dot(zz[0], gd0_v[...], preferred_element_type=f32)
        e1 = jnp.dot(zz[1], gd_v[0:256, :], preferred_element_type=f32)
        e2 = jnp.dot(zz[2], gd_v[256:512, :], preferred_element_type=f32)
        e1r, e1i, e2r, e2i = e1[:, 0:128], e1[:, 128:256], e2[:, 0:128], e2[:, 128:256]
        p1 = c0 + C5[0] * e1r + C5[1] * e2r
        q1 = S5[0] * e1i + S5[1] * e2i
        p2 = c0 + C5[1] * e1r + C5[0] * e2r
        q2 = S5[1] * e1i - S5[0] * e2i
        ys = (c0 + e1r + e2r, p1 - q1, p2 - q2, p2 + q2, p1 + q1)
        for t in range(5):
            sta_s[pl.ds(r, CH), 128 * t:128 * (t + 1)] = ys[t].astype(bf16)
        outa_copy(c).start()
        return carry

    jax.lax.fori_loop(0, NCH, irfft_body, 0)

    c_wo.wait()

    def oproj_body(c, carry):
        r = pl.multiple_of(c * CO, CO)
        stb_s[pl.ds(r, CO), :] = jnp.dot(
            o_s[pl.ds(r, CO), :], wo_v[...], preferred_element_type=f32).astype(bf16)
        outb_copy(c).start()
        return carry

    jax.lax.fori_loop(0, NCO, oproj_body, 0)

    for c in range(NCO):
        outb_copy(c).wait()
    for c in range(NCH):
        outa_copy(c).wait()


@jax.jit
def pallas_concat_heads__spectral_gfnet__sliding_block__prompt_kernel(
    A_x, A_w_r, A_w_i, B_x, B_wqkv, B_wo,
):
    bf16 = jnp.bfloat16
    f32 = jnp.float32
    fd, gd0, gd, ff, fi, twr, twi = _make_consts()
    xa = A_x.reshape(S, D)
    xb = B_x.reshape(S, D)
    any_spec = pl.BlockSpec(memory_space=pltpu.MemorySpace.HBM)
    out = pl.pallas_call(
        _kernel,
        out_shape=jax.ShapeDtypeStruct((S, 2 * D), bf16),
        in_specs=[any_spec] * 13,
        out_specs=any_spec,
        scratch_shapes=[
            pltpu.VMEM((S, D), bf16),
            pltpu.VMEM((D, 3 * D), bf16),
            pltpu.VMEM((D, D), bf16),
            pltpu.VMEM((S, D), bf16),
            pltpu.VMEM((DF, S), bf16),
            pltpu.VMEM((DF, S), bf16),
            pltpu.VMEM((D, 256), bf16),
            pltpu.VMEM((256, 128), bf16),
            pltpu.VMEM((512, 256), bf16),
            pltpu.VMEM((2 * N2, 2 * N2), bf16),
            pltpu.VMEM((2 * N2, 2 * N2), bf16),
            pltpu.VMEM((S, 128), f32),
            pltpu.VMEM((S, 128), f32),
            pltpu.VMEM((S, DX), f32),
            pltpu.VMEM((S + WIN, DX), bf16),
            pltpu.VMEM(((S + WIN) // 128, H * HP, 128), bf16),
            pltpu.VMEM((H, KW, QB), f32),
            pltpu.VMEM((H, KW, QB), f32),
            pltpu.VMEM((H, 8, QB), f32),
            pltpu.VMEM((H, 8, QB), f32),
            pltpu.VMEM((D, 128), f32),
            pltpu.VMEM((S, D), bf16),
            pltpu.VMEM((S, 2 * DFP), f32),
            pltpu.VMEM((N1, 2 * N2, DFP), f32),
            pltpu.VMEM((WPU, D, 128), f32),
            pltpu.VMEM((3, S, 128), f32),
            pltpu.VMEM((3, S, 128), f32),
            pltpu.VMEM((S, D), bf16),
            pltpu.VMEM((S, D), bf16),
            pltpu.SemaphoreType.DMA((14,)),
            pltpu.SemaphoreType.DMA((NCH,)),
            pltpu.SemaphoreType.DMA((NCH,)),
            pltpu.SemaphoreType.DMA((NCO,)),
        ],
        compiler_params=pltpu.CompilerParams(
            vmem_limit_bytes=110 * 1024 * 1024),
    )(xb, B_wqkv, B_wo, xa, A_w_r.T, A_w_i.T, fd, gd0, gd, ff, fi, twr, twi)
    return out.reshape(1, S, 2 * D)
```
